```python
import os as _os
_os.environ.setdefault("JAX_PLATFORMS", "cpu")
import jax
import jax.numpy as jnp

def _softmax(x, axis=-1):
    return jax.nn.softmax(x, axis=axis)
def _gelu(x):
    return jax.nn.gelu(x, approximate=True)
def _silu(x):
    return jax.nn.silu(x)
def _sigmoid(x):
    return jax.nn.sigmoid(x)
def _layernorm(x, axis=-1, eps=1e-5):
    m = jnp.mean(x, axis=axis, keepdims=True)
    v = jnp.var(x, axis=axis, keepdims=True)
    return (x - m) / jnp.sqrt(v + eps)
def _scatter_add(tgt, idx, src, axis=0):
    return tgt.at[idx].add(src)
def _segment_sum(src, seg, n):
    return jax.ops.segment_sum(src, seg, n)
class _Rng:
    def __init__(self, key):
        self._k = key
    def _next(self):
        self._k, sub = jax.random.split(self._k)
        return sub
    def normal(self, shape):
        return jax.random.normal(self._next(), shape, dtype=jnp.bfloat16)
    def randint(self, lo, hi, shape):
        return jax.random.randint(self._next(), shape, lo, hi, dtype=jnp.int32)
    def uniform(self, shape, lo=0.0, hi=1.0):
        return jax.random.uniform(self._next(), shape, jnp.bfloat16, lo, hi)
    def permutation(self, n):
        return jax.random.permutation(self._next(), n)


kernel_name = 'gated_mix__mha_block__softmax_full_mha__prompt'

def setup_inputs():
    _rng = _Rng(jax.random.key(int.from_bytes(__import__("os").urandom(4), "little")))
    _w = (lambda a: (lambda t: t.astype(jnp.bfloat16) if jnp.issubdtype(t.dtype, jnp.floating) else t)(jnp.asarray(a)))
    def _A_setup():
        B, S, D, H = 1, 2048, 448, 16
        return {
            "x": _w((lambda *s: _rng.normal(s) * 0.05)(B, S, D)),
            "wqkv": _w((lambda *s: _rng.normal(s) * 0.4)(D, 3 * D)),
            "wo": _w((lambda *s: _rng.normal(s) * 0.05)(D, D)),
        }
    _A_in = _A_setup()

    def _B_setup():
        B, S, D = 1, 2048, 448
        return {
            "x": _w((lambda *s: _rng.normal(s) * 0.05)(B, S, D)),
            "wqkv": _w((lambda *s: _rng.normal(s) * 0.4)(D, 3 * D)),
            "wo": _w((lambda *s: _rng.normal(s) * 0.05)(D, D)),
        }
    _B_in = _B_setup()

    return {
        "A_x": _A_in["x"],
        "A_wqkv": _A_in["wqkv"],
        "A_wo": _A_in["wo"],
        "B_x": _B_in["x"],
        "B_wqkv": _B_in["wqkv"],
        "B_wo": _B_in["wo"],
        "gate_w": _w((lambda *s: _rng.normal(s) * 0.05)(448) * 16.0),
    }

def reference(A_x, A_wqkv, A_wo, B_x, B_wqkv, B_wo, gate_w):
    def _A_ref(x, wqkv, wo):
        B, S, D = x.shape
        H = 16
        Dh = D // H
        qkv = (lambda x, *d: x.transpose(*d))((x @ wqkv).reshape(B, S, 3, H, Dh), 2, 0, 3, 1, 4)
        q, k, v = qkv[0], qkv[1], qkv[2]
        scores = jnp.einsum("bhqd,bhkd->bhqk", q, k) * (Dh ** -0.5)
        p = _softmax(scores, axis=-1)
        o = jnp.einsum("bhqk,bhkd->bhqd", p, v)
        return (lambda x, *d: x.transpose(*d))(o, 0, 2, 1, 3).reshape(B, S, D) @ wo

    def _B_ref(x, wqkv, wo):
        B, S, D = x.shape
        H = 16; Dh = D // H
        qkv = (lambda x, *d: x.transpose(*d))((x @ wqkv).reshape(B, S, 3, H, Dh), 2, 0, 3, 1, 4)
        q, k, v = qkv[0], qkv[1], qkv[2]
        scale = Dh ** -0.5
        scores = jnp.einsum("bhqd,bhkd->bhqk", q, k) * scale
        p = _softmax(scores, axis=-1)
        o = jnp.einsum("bhqk,bhkd->bhqd", p, v)
        return (lambda x, *d: x.transpose(*d))(o, 0, 2, 1, 3).reshape(B, S, D) @ wo

    x = A_x
    g = _sigmoid((x * gate_w).sum(-1, keepdims=True))
    a = _A_ref(x, A_wqkv, A_wo)
    b = _B_ref(x, B_wqkv, B_wo)
    return g * a + (1 - g) * b
```

```python
import functools, math
import jax
import jax.numpy as jnp
import jax.experimental.pallas as pl
import jax.experimental.pallas.tpu as pltpu

S = 2048
D = 448
H = 16
DH = 28
DP = 32
GW = 4 * DH
NG = 8
NH = 32
QSCALE = (DH ** -0.5) * math.log2(math.e)
NT_DIMS = (((1,), (1,)), ((), ()))
TT_DIMS = (((0,), (1,)), ((), ()))
TN_DIMS = (((0,), (0,)), ((), ()))


def make(TQ=512, TK=256):
    NQ = S // TQ
    NC = S // TK
    NI = NQ * NG

    def kernel(x_ref, wa_ref, wb_ref, woa_ref, wob_ref, gw_ref, o_ref,
               k_scr, qT_scr, vT_scr, oT_scr, sA, sB, gate_scr, wo_scr):
        xT = x_ref[...]
        x = xT.T
        wo_scr[0:D, :] = woa_ref[...]
        wo_scr[D:2 * D, :] = wob_ref[...]
        tail = jnp.where(jax.lax.broadcasted_iota(jnp.int32, (DP - DH, S), 0) == 0, 1.0, 0.0)
        for b, w_ref in enumerate((wa_ref, wb_ref)):
            for g in range(4):
                G = 4 * b + g
                wk = w_ref[:, D + GW * g: D + GW * g + 128]
                k_scr[G] = jnp.dot(x, wk, preferred_element_type=jnp.float32).astype(jnp.bfloat16)
                wq = w_ref[:, GW * g: GW * g + 128]
                qt = jax.lax.dot_general(wq, xT, TN_DIMS, preferred_element_type=jnp.float32) * QSCALE
                for qi in range(NQ):
                    qT_scr[qi, G] = qt[:, qi * TQ:(qi + 1) * TQ]
                v0 = min(2 * D + GW * g, 3 * D - 128)
                off = 2 * D + GW * g - v0
                wv = w_ref[:, v0: v0 + 128]
                vt = jax.lax.dot_general(wv, xT, TN_DIMS, preferred_element_type=jnp.float32)
                for j in range(4):
                    piece = vt[off + DH * j: off + DH * (j + 1), :]
                    vT_scr[4 * G + j] = jnp.concatenate([piece, tail], axis=0).astype(jnp.bfloat16)
        gw8 = jnp.broadcast_to(gw_ref[...], (8, D))
        glog = jnp.dot(gw8, xT, preferred_element_type=jnp.float32)
        gate = jax.nn.sigmoid(glog)
        for qi in range(NQ):
            gate_scr[qi] = gate[:, qi * TQ:(qi + 1) * TQ]

        row = jax.lax.broadcasted_iota(jnp.int32, (128, TQ), 0)

        def masked_q(i, j):
            qT = qT_scr[i // NG, i % NG]
            return jnp.where((row >= j * DH) & (row < (j + 1) * DH), qT, 0.0).astype(jnp.bfloat16)

        def stage1(qm, G, buf, c, m8):
            kc = k_scr[G, c * TK:(c + 1) * TK, :]
            sT = jnp.dot(kc, qm, preferred_element_type=jnp.float32)
            buf[c * TK:(c + 1) * TK, :] = sT
            mc = jnp.max(sT.reshape(TK // 8, 8, TQ), axis=0)
            return mc if m8 is None else jnp.maximum(m8, mc)

        def stage2(h, buf, c, m, acc):
            sT = buf[c * TK:(c + 1) * TK, :]
            pT = jnp.exp2(sT - m).astype(jnp.bfloat16)
            vt = vT_scr[h, :, c * TK:(c + 1) * TK]
            o = jnp.dot(vt, pT, preferred_element_type=jnp.float32)
            return o if acc is None else acc + o

        qm = masked_q(0, 0)
        m8 = None
        for c in range(NC):
            m8 = stage1(qm, 0, sA, c, m8)
        m0 = jnp.max(m8, axis=0, keepdims=True)

        def body(i, m):
            qi = i // NG
            G = i % NG
            gate = gate_scr[qi][0:1, :]
            gsel = jnp.where(G < NG // 2, gate, 1.0 - gate)
            outs = []
            for j in range(4):
                rd, wr = (sA, sB) if j % 2 == 0 else (sB, sA)
                if j < 3:
                    inext, jn = i, j + 1
                else:
                    inext, jn = jnp.minimum(i + 1, NI - 1), 0
                qm = masked_q(inext, jn)
                Gn = inext % NG
                m8 = None
                acc = None
                for c in range(NC):
                    m8 = stage1(qm, Gn, wr, c, m8)
                    acc = stage2(4 * G + j, rd, c, m, acc)
                l = acc[DH:DH + 1, :]
                outs.append(acc[0:DH, :] * (gsel / l))
                m = jnp.max(m8, axis=0, keepdims=True)
            og = jnp.concatenate(outs, axis=0).astype(jnp.bfloat16)
            oT_scr[qi, pl.ds(pl.multiple_of(G * GW, 16), GW), :] = og
            return m

        jax.lax.fori_loop(0, NI, body, m0)

        for qi in range(NQ):
            outT = jax.lax.dot_general(wo_scr[...], oT_scr[qi], TN_DIMS, preferred_element_type=jnp.float32)
            o_ref[:, qi * TQ:(qi + 1) * TQ] = outT.astype(o_ref.dtype)

    def fn(A_x, A_wqkv, A_wo, B_x, B_wqkv, B_wo, gate_w):
        x = A_x.reshape(S, D).T
        gw = gate_w.reshape(1, D)
        out = pl.pallas_call(
            kernel,
            out_shape=jax.ShapeDtypeStruct((D, S), jnp.bfloat16),
            scratch_shapes=[pltpu.VMEM((NG, S, 128), jnp.bfloat16),
                            pltpu.VMEM((NQ, NG, 128, TQ), jnp.float32),
                            pltpu.VMEM((NH, DP, S), jnp.bfloat16),
                            pltpu.VMEM((NQ, 2 * D, TQ), jnp.bfloat16),
                            pltpu.VMEM((S, TQ), jnp.float32),
                            pltpu.VMEM((S, TQ), jnp.float32),
                            pltpu.VMEM((NQ, 8, TQ), jnp.float32),
                            pltpu.VMEM((2 * D, D), jnp.bfloat16)],
            compiler_params=pltpu.CompilerParams(
                vmem_limit_bytes=100 * 1024 * 1024),
        )(x, A_wqkv, B_wqkv, A_wo, B_wo, gw)
        return out.T.reshape(1, S, D)
    return fn


_impl = make(TQ=512, TK=256)


@jax.jit
def pallas_gated_mix__mha_block__softmax_full_mha__prompt_kernel(
    A_x: jax.Array,
    A_wqkv: jax.Array,
    A_wo: jax.Array,
    B_x: jax.Array,
    B_wqkv: jax.Array,
    B_wo: jax.Array,
    gate_w: jax.Array,
):
    return _impl(A_x, A_wqkv, A_wo, B_x, B_wqkv, B_wo, gate_w)
```

```python
import functools, math
import jax
import jax.numpy as jnp
import jax.experimental.pallas as pl
import jax.experimental.pallas.tpu as pltpu

S = 2048
D = 448
H = 16
DH = 28
DP = 32
GW = 4 * DH
NG = 8
NH = 32
QSCALE = (DH ** -0.5) * math.log2(math.e)
TN_DIMS = (((0,), (0,)), ((), ()))


def make(TQ=1024, TK=128):
    NQ = S // TQ
    NC = S // TK
    NI = NQ * NG

    def kernel(x_ref, wa_ref, wb_ref, woa_ref, wob_ref, gw_ref, o_ref,
               k_scr, qT_scr, vT_scr, oT_scr, s_scr, gate_scr, wo_scr):
        sA = s_scr.at[0]
        sB = s_scr.at[1]
        xT = x_ref[...]
        x = xT.T
        wo_scr[0:D, :] = woa_ref[...]
        wo_scr[D:2 * D, :] = wob_ref[...]
        tail = jnp.where(jax.lax.broadcasted_iota(jnp.int32, (DP - DH, S), 0) == 0, 1.0, 0.0)
        for b, w_ref in enumerate((wa_ref, wb_ref)):
            for g in range(4):
                G = 4 * b + g
                wk = w_ref[:, D + GW * g: D + GW * g + 128]
                k_scr[G] = jnp.dot(x, wk, preferred_element_type=jnp.float32).astype(jnp.bfloat16)
                wq = w_ref[:, GW * g: GW * (g + 1)]
                qt = jax.lax.dot_general(wq, xT, TN_DIMS, preferred_element_type=jnp.float32) * QSCALE
                for qi in range(NQ):
                    qT_scr[qi, G] = qt[:, qi * TQ:(qi + 1) * TQ]
                wv = w_ref[:, 2 * D + GW * g: 2 * D + GW * (g + 1)]
                vt = jax.lax.dot_general(wv, xT, TN_DIMS, preferred_element_type=jnp.float32)
                for j in range(4):
                    piece = vt[DH * j: DH * (j + 1), :]
                    vT_scr[4 * G + j] = jnp.concatenate([piece, tail], axis=0).astype(jnp.bfloat16)
        gw8 = jnp.broadcast_to(gw_ref[...], (8, D))
        glog = jnp.dot(gw8, xT, preferred_element_type=jnp.float32)
        gate = jax.nn.sigmoid(glog)
        for qi in range(NQ):
            gate_scr[qi] = gate[:, qi * TQ:(qi + 1) * TQ]

        row = jax.lax.broadcasted_iota(jnp.int32, (GW, TQ), 0)
        zpad = jnp.zeros((128 - GW, TQ), jnp.float32)

        def masked_q(i, j):
            qT = qT_scr[i // NG, i % NG]
            qm = jnp.where((row >= j * DH) & (row < (j + 1) * DH), qT, 0.0)
            return jnp.concatenate([qm, zpad], axis=0).astype(jnp.bfloat16)

        def stage1(qm, G, buf, c):
            kc = k_scr[G, c * TK:(c + 1) * TK, :]
            sT = jnp.dot(kc, qm, preferred_element_type=jnp.float32)
            buf[...] = sT
            return jnp.max(sT, axis=0, keepdims=True)

        def stage2(h, buf, c, mc, m_run, acc):
            m_new = mc if m_run is None else jnp.maximum(m_run, mc)
            pT = jnp.exp2(buf[...] - m_new).astype(jnp.bfloat16)
            vt = vT_scr[h, :, c * TK:(c + 1) * TK]
            o = jnp.dot(vt, pT, preferred_element_type=jnp.float32)
            if acc is not None:
                o = acc * jnp.exp2(m_run - m_new) + o
            return m_new, o

        qm0 = masked_q(0, 0)
        mc0 = stage1(qm0, 0, sA, 0)

        def body(i, mc):
            qi = i // NG
            G = i % NG
            gate = gate_scr[qi][0:1, :]
            gsel = jnp.where(G < NG // 2, gate, 1.0 - gate)
            outs = []
            qm = masked_q(i, 0)
            for j in range(4):
                m_run = None
                acc = None
                for c in range(NC):
                    rd, wr = (sA, sB) if c % 2 == 0 else (sB, sA)
                    if c < NC - 1:
                        mcn = stage1(qm, G, wr, c + 1)
                    else:
                        if j < 3:
                            inext, jn = i, j + 1
                        else:
                            inext, jn = jnp.minimum(i + 1, NI - 1), 0
                        qm = masked_q(inext, jn)
                        mcn = stage1(qm, inext % NG, wr, 0)
                    m_run, acc = stage2(4 * G + j, rd, c, mc, m_run, acc)
                    mc = mcn
                l = acc[DH:DH + 1, :]
                outs.append(acc[0:DH, :] * (gsel / l))
            og = jnp.concatenate(outs, axis=0).astype(jnp.bfloat16)
            oT_scr[qi, pl.ds(pl.multiple_of(G * GW, 16), GW), :] = og
            return mc

        jax.lax.fori_loop(0, NI, body, mc0)

        for qi in range(NQ):
            outT = jax.lax.dot_general(wo_scr[...], oT_scr[qi], TN_DIMS, preferred_element_type=jnp.float32)
            o_ref[:, qi * TQ:(qi + 1) * TQ] = outT.astype(o_ref.dtype)

    def fn(A_x, A_wqkv, A_wo, B_x, B_wqkv, B_wo, gate_w):
        x = A_x.reshape(S, D).T
        gw = gate_w.reshape(1, D)
        out = pl.pallas_call(
            kernel,
            out_shape=jax.ShapeDtypeStruct((D, S), jnp.bfloat16),
            scratch_shapes=[pltpu.VMEM((NG, S, 128), jnp.bfloat16),
                            pltpu.VMEM((NQ, NG, GW, TQ), jnp.float32),
                            pltpu.VMEM((NH, DP, S), jnp.bfloat16),
                            pltpu.VMEM((NQ, 2 * D, TQ), jnp.bfloat16),
                            pltpu.VMEM((2, TK, TQ), jnp.float32),
                            pltpu.VMEM((NQ, 8, TQ), jnp.float32),
                            pltpu.VMEM((2 * D, D), jnp.bfloat16)],
            compiler_params=pltpu.CompilerParams(
                vmem_limit_bytes=100 * 1024 * 1024),
        )(x, A_wqkv, B_wqkv, A_wo, B_wo, gw)
        return out.T.reshape(1, S, D)
    return fn


_impl = make(TQ=1024, TK=128)


@jax.jit
def pallas_gated_mix__mha_block__softmax_full_mha__prompt_kernel(
    A_x: jax.Array,
    A_wqkv: jax.Array,
    A_wo: jax.Array,
    B_x: jax.Array,
    B_wqkv: jax.Array,
    B_wo: jax.Array,
    gate_w: jax.Array,
):
    return _impl(A_x, A_wqkv, A_wo, B_x, B_wqkv, B_wo, gate_w)
```

```python
import math

import jax
import jax.numpy as jnp
import jax.experimental.pallas as pl
import jax.experimental.pallas.tpu as pltpu

S = 2048
D = 448
H = 16
DH = 28
DP = 32
GW = 4 * DH
NG = 8
NH = 32
QSCALE = (DH ** -0.5) * math.log2(math.e)
TN_DIMS = (((0,), (0,)), ((), ()))


def make(TQ=1024, TK=128):
    NQ = S // TQ
    NC = S // TK
    NI = NQ * NG
    HS = S // 2
    NO = 4
    TO = S // NO

    def kernel(x_hbm, wa_hbm, wb_hbm, woa_hbm, wob_hbm, gw_ref, o_hbm,
               k_scr, qT_scr, vT_scr, oT_scr, s_scr, gate_scr, wo_scr,
               x_ref, wa_ref, wb_ref, o_ref, wqa_ref, sems):
        sA = s_scr.at[0]
        sB = s_scr.at[1]
        cp_x = [pltpu.make_async_copy(x_hbm.at[:, n * HS:(n + 1) * HS],
                                      x_ref.at[:, n * HS:(n + 1) * HS],
                                      sems.at[n]) for n in range(2)]
        cp_wa = [pltpu.make_async_copy(wa_hbm.at[:, 0:512], wqa_ref, sems.at[2]),
                 pltpu.make_async_copy(wa_hbm, wa_ref, sems.at[3])]
        cp_wb = pltpu.make_async_copy(wb_hbm, wb_ref, sems.at[4])
        cp_woa = pltpu.make_async_copy(woa_hbm, wo_scr.at[0:D, :], sems.at[5])
        cp_wob = pltpu.make_async_copy(wob_hbm, wo_scr.at[D:2 * D, :], sems.at[6])
        cp_x[0].start()
        cp_wa[0].start()
        cp_x[1].start()
        cp_wa[1].start()
        cp_wb.start()
        cp_woa.start()
        cp_wob.start()
        tail = jnp.where(jax.lax.broadcasted_iota(jnp.int32, (DP - DH, S), 0) == 0, 1.0, 0.0)

        def proj_q(w_ref, b, n):
            xh = x_ref[:, n * HS:(n + 1) * HS]
            for g in range(4):
                wq = w_ref[:, GW * g: GW * (g + 1)]
                qt = jax.lax.dot_general(wq, xh, TN_DIMS, preferred_element_type=jnp.float32) * QSCALE
                for r in range(HS // TQ):
                    qT_scr[n * (HS // TQ) + r, 4 * b + g] = qt[:, r * TQ:(r + 1) * TQ]

        def proj_v(w_ref, b, xT):
            for g in range(4):
                G = 4 * b + g
                wv = w_ref[:, 2 * D + GW * g: 2 * D + GW * (g + 1)]
                vt = jax.lax.dot_general(wv, xT, TN_DIMS, preferred_element_type=jnp.float32)
                for j in range(4):
                    piece = vt[DH * j: DH * (j + 1), :]
                    vT_scr[4 * G + j] = jnp.concatenate([piece, tail], axis=0).astype(jnp.bfloat16)

        def proj_k(w_ref, b, x):
            for g in range(4):
                wk = w_ref[:, D + GW * g: D + GW * g + 128]
                k_scr[4 * b + g] = jnp.dot(x, wk, preferred_element_type=jnp.float32).astype(jnp.bfloat16)

        cp_x[0].wait()
        cp_wa[0].wait()
        proj_q(wqa_ref, 0, 0)
        cp_x[1].wait()
        proj_q(wqa_ref, 0, 1)
        xT = x_ref[...]
        cp_wa[1].wait()
        proj_v(wa_ref, 0, xT)
        x = xT.T
        proj_k(wa_ref, 0, x)
        cp_wb.wait()
        proj_q(wb_ref, 1, 0)
        proj_q(wb_ref, 1, 1)
        proj_v(wb_ref, 1, xT)
        proj_k(wb_ref, 1, x)
        gw8 = jnp.broadcast_to(gw_ref[...], (8, D))
        glog = jnp.dot(gw8, xT, preferred_element_type=jnp.float32)
        gate = jax.nn.sigmoid(glog)
        for qi in range(NQ):
            gate_scr[qi] = gate[:, qi * TQ:(qi + 1) * TQ]

        row = jax.lax.broadcasted_iota(jnp.int32, (GW, TQ), 0)
        zpad = jnp.zeros((128 - GW, TQ), jnp.float32)

        def masked_q(i, j):
            qT = qT_scr[i // NG, i % NG]
            qm = jnp.where((row >= j * DH) & (row < (j + 1) * DH), qT, 0.0)
            return jnp.concatenate([qm, zpad], axis=0).astype(jnp.bfloat16)

        def stage1(qm, G, buf, c):
            kc = k_scr[G, c * TK:(c + 1) * TK, :]
            sT = jnp.dot(kc, qm, preferred_element_type=jnp.float32)
            buf[...] = sT
            return jnp.max(sT, axis=0, keepdims=True)

        def stage2(h, buf, c, mc, m_run, acc):
            m_new = mc if m_run is None else jnp.maximum(m_run, mc)
            pT = jnp.exp2(buf[...] - m_new).astype(jnp.bfloat16)
            vt = vT_scr[h, :, c * TK:(c + 1) * TK]
            o = jnp.dot(vt, pT, preferred_element_type=jnp.float32)
            if acc is not None:
                o = acc * jnp.exp2(m_run - m_new) + o
            return m_new, o

        qm0 = masked_q(0, 0)
        mc0 = stage1(qm0, 0, sA, 0)

        def body(i, mc):
            qi = i // NG
            G = i % NG
            gate = gate_scr[qi][0:1, :]
            gsel = jnp.where(G < NG // 2, gate, 1.0 - gate)
            outs = []
            qm = masked_q(i, 0)
            for j in range(4):
                m_run = None
                acc = None
                for c in range(NC):
                    rd, wr = (sA, sB) if c % 2 == 0 else (sB, sA)
                    if c < NC - 1:
                        mcn = stage1(qm, G, wr, c + 1)
                    else:
                        if j < 3:
                            inext, jn = i, j + 1
                        else:
                            inext, jn = jnp.minimum(i + 1, NI - 1), 0
                        qm = masked_q(inext, jn)
                        mcn = stage1(qm, inext % NG, wr, 0)
                    m_run, acc = stage2(4 * G + j, rd, c, mc, m_run, acc)
                    mc = mcn
                l = acc[DH:DH + 1, :]
                outs.append(acc[0:DH, :] * (gsel / l))
            og = jnp.concatenate(outs, axis=0).astype(jnp.bfloat16)
            oT_scr[qi, pl.ds(pl.multiple_of(G * GW, 16), GW), :] = og
            return mc

        jax.lax.fori_loop(0, NI, body, mc0)

        cp_woa.wait()
        cp_wob.wait()
        cps = []
        for oi in range(NO):
            qi, r = divmod(oi * TO, TQ)
            outT = jax.lax.dot_general(wo_scr[...], oT_scr[qi, :, r:r + TO], TN_DIMS,
                                       preferred_element_type=jnp.float32)
            o_ref[:, oi * TO:(oi + 1) * TO] = outT.astype(o_ref.dtype)
            cp = pltpu.make_async_copy(o_ref.at[:, oi * TO:(oi + 1) * TO],
                                       o_hbm.at[:, oi * TO:(oi + 1) * TO], sems.at[7 + oi])
            cp.start()
            cps.append(cp)
        for cp in cps:
            cp.wait()

    def fn(A_x, A_wqkv, A_wo, B_x, B_wqkv, B_wo, gate_w):
        x = A_x.reshape(S, D).T
        gw = gate_w.reshape(1, D)
        out = pl.pallas_call(
            kernel,
            out_shape=jax.ShapeDtypeStruct((D, S), jnp.bfloat16),
            in_specs=[pl.BlockSpec(memory_space=pl.ANY)] * 5 + [pl.BlockSpec(memory_space=pltpu.VMEM)],
            out_specs=pl.BlockSpec(memory_space=pl.ANY),
            scratch_shapes=[pltpu.VMEM((NG, S, 128), jnp.bfloat16),
                            pltpu.VMEM((NQ, NG, GW, TQ), jnp.float32),
                            pltpu.VMEM((NH, DP, S), jnp.bfloat16),
                            pltpu.VMEM((NQ, 2 * D, TQ), jnp.bfloat16),
                            pltpu.VMEM((2, TK, TQ), jnp.float32),
                            pltpu.VMEM((NQ, 8, TQ), jnp.float32),
                            pltpu.VMEM((2 * D, D), jnp.bfloat16),
                            pltpu.VMEM((D, S), jnp.bfloat16),
                            pltpu.VMEM((D, 3 * D), jnp.bfloat16),
                            pltpu.VMEM((D, 3 * D), jnp.bfloat16),
                            pltpu.VMEM((D, S), jnp.bfloat16),
                            pltpu.VMEM((D, 512), jnp.bfloat16),
                            pltpu.SemaphoreType.DMA((7 + NO,))],
            compiler_params=pltpu.CompilerParams(
                vmem_limit_bytes=100 * 1024 * 1024),
        )(x, A_wqkv, B_wqkv, A_wo, B_wo, gw)
        return out.T.reshape(1, S, D)
    return fn


_impl = make()


@jax.jit
def pallas_gated_mix__mha_block__softmax_full_mha__prompt_kernel(
    A_x: jax.Array,
    A_wqkv: jax.Array,
    A_wo: jax.Array,
    B_x: jax.Array,
    B_wqkv: jax.Array,
    B_wo: jax.Array,
    gate_w: jax.Array,
):
    return _impl(A_x, A_wqkv, A_wo, B_x, B_wqkv, B_wo, gate_w)
```
